```python
import jax
import jax.numpy as jnp

def _softmax(x, axis=-1):
    return jax.nn.softmax(x, axis=axis)
def _gelu(x):
    return jax.nn.gelu(x, approximate=True)
def _silu(x):
    return jax.nn.silu(x)
def _sigmoid(x):
    return jax.nn.sigmoid(x)
def _layernorm(x, axis=-1, eps=1e-5):
    m = jnp.mean(x, axis=axis, keepdims=True)
    v = jnp.var(x, axis=axis, keepdims=True)
    return (x - m) / jnp.sqrt(v + eps)
def _scatter_add(tgt, idx, src, axis=0):
    return tgt.at[idx].add(src)
def _segment_sum(src, seg, n):
    return jax.ops.segment_sum(src, seg, n)
class _Rng:
    def __init__(self, key):
        self._k = key
    def _next(self):
        self._k, sub = jax.random.split(self._k)
        return sub
    def normal(self, shape):
        return jax.random.normal(self._next(), shape, dtype=jnp.bfloat16)
    def randint(self, lo, hi, shape):
        return jax.random.randint(self._next(), shape, lo, hi, dtype=jnp.int32)
    def uniform(self, shape, lo=0.0, hi=1.0):
        return jax.random.uniform(self._next(), shape, jnp.bfloat16, lo, hi)
    def permutation(self, n):
        return jax.random.permutation(self._next(), n)


kernel_name = 'recurrent_scan__sliding_block_cached__mixer_s_mlp__decode'

def setup_inputs():
    _rng = _Rng(jax.random.key(int.from_bytes(__import__("os").urandom(4), "little")))
    _w = (lambda a: (lambda t: t.astype(jnp.bfloat16) if jnp.issubdtype(t.dtype, jnp.floating) else t)(jnp.asarray(a)))
    def _A_setup():
        B, Sq, D = 1, 1, 512
        Hq, Hkv, Sk, Dh = 32, 32, 32768, 128
        assert Hq % Hkv == 0, (Hq, Hkv)
        return {
            "x": _w((lambda *s: _rng.normal(s) * 0.05)(B, Sq, D)),
            "k_cache": _w((lambda *s: _rng.normal(s) * 0.05)(B, Hkv, Sk, Dh)),
            "v_cache": _w((lambda *s: _rng.normal(s) * 0.05)(B, Hkv, Sk, Dh)),
            "wq": _w((lambda *s: _rng.normal(s) * 0.05)(D, Hq * Dh) * (D ** -0.5)),
            "wo": _w((lambda *s: _rng.normal(s) * 0.05)(Hq * Dh, D) * ((Hq * Dh) ** -0.5)),
        }
    _A_in = _A_setup()

    def _B_setup():
        B, S, D, F = 1, 1, 512, 1376
        return {
            "x":  _w((lambda *s: _rng.normal(s) * 0.05)(B, S, D)),
            "w1": _w((lambda *s: _rng.normal(s) * 0.05)(D, D) * (D ** -0.5)),
            "w2": _w((lambda *s: _rng.normal(s) * 0.05)(D, D) * (D ** -0.5)),
            "w3": _w((lambda *s: _rng.normal(s) * 0.05)(D, F) * (D ** -0.5)),
            "w4": _w((lambda *s: _rng.normal(s) * 0.05)(F, D) * (F ** -0.5)),
        }
    _B_in = _B_setup()

    return {
        "A_x": _A_in["x"],
        "A_k_cache": _A_in["k_cache"],
        "A_v_cache": _A_in["v_cache"],
        "A_wq": _A_in["wq"],
        "A_wo": _A_in["wo"],
        "B_x": _B_in["x"],
        "B_w1": _B_in["w1"],
        "B_w2": _B_in["w2"],
        "B_w3": _B_in["w3"],
        "B_w4": _B_in["w4"],
    }

def reference(A_x, A_k_cache, A_v_cache, A_wq, A_wo, B_x, B_w1, B_w2, B_w3, B_w4):
    def _A_ref(x, k_cache, v_cache, wq, wo):
        B, Sq, D = x.shape
        Hq, Dh = 32, 128
        Hkv, Sk = k_cache.shape[1], k_cache.shape[2]
        W = min(4096, max(256, Sk // 4))
        rep = Hq // Hkv
        q = (lambda x, *d: x.transpose(*d))((x @ wq).reshape(B, Sq, Hq, Dh), 0, 2, 1, 3)
        k = jnp.repeat(k_cache[:, :, Sk - W:, :], rep, axis=1)
        v = jnp.repeat(v_cache[:, :, Sk - W:, :], rep, axis=1)
        scores = jnp.einsum("bhqd,bhkd->bhqk", q, k) * (Dh ** -0.5)
        p = _softmax(scores, axis=-1)
        o = jnp.einsum("bhqk,bhkd->bhqd", p, v)
        return (lambda x, *d: x.transpose(*d))(o, 0, 2, 1, 3).reshape(B, Sq, Hq * Dh) @ wo

    def _B_ref(x, w1, w2, w3, w4):
        B, S, D = x.shape
        h = _gelu(_layernorm(x, axis=-1) @ w1)
        c = D // 4
        g0 = jnp.pad(h[:, :, 0*c:1*c], ((0, 0), (1, 0), (0, 0)))[:, :S, :]
        g1 = jnp.pad(h[:, :, 1*c:2*c], ((0, 0), (0, 1), (0, 0)))[:, 1:, :]
        g2 = jnp.pad(h[:, :, 2*c:3*c], ((0, 0), (2, 0), (0, 0)))[:, :S, :]
        g3 = jnp.pad(h[:, :, 3*c:   ], ((0, 0), (0, 2), (0, 0)))[:, 2:, :]
        hs = jnp.concatenate([g0, g1, g2, g3], axis=-1) @ w2
        x1 = x + hs
        h2 = _gelu(_layernorm(x1, axis=-1) @ w3) @ w4
        return x1 + h2

    x = A_x
    xn = _layernorm(x, axis=-1)
    s = _A_ref(xn, A_k_cache, A_v_cache, A_wq, A_wo)
    g = _silu(_B_ref(xn, B_w1, B_w2, B_w3, B_w4))
    return x + s * g
```

```python
import jax
import jax.numpy as jnp
from jax import lax
from jax.experimental import pallas as pl
from jax.experimental.pallas import tpu as pltpu

D = 512
H = 32
DH = 128
F = 1376
BF = jnp.bfloat16
F32 = jnp.float32
LOG2E = 1.4426950408889634
NT = (((1,), (1,)), ((), ()))

G = 8
WO_CHUNKS = (8, 8, 8, 4, 2, 1, 1)


def _ln(x, eps=1e-5):
    m = jnp.mean(x, axis=-1, keepdims=True)
    xc = x - m
    v = jnp.mean(xc * xc, axis=-1, keepdims=True)
    return xc * lax.rsqrt(v + eps)


@jax.jit
def pallas_recurrent_scan__sliding_block_cached__mixer_s_mlp__decode_kernel(
    A_x: jax.Array,
    A_k_cache: jax.Array,
    A_v_cache: jax.Array,
    A_wq: jax.Array,
    A_wo: jax.Array,
    B_x: jax.Array,
    B_w1: jax.Array,
    B_w2: jax.Array,
    B_w3: jax.Array,
    B_w4: jax.Array,
):
    assert A_x.shape == (1, 1, D)
    SK = A_k_cache.shape[2]
    W = min(4096, max(256, SK // 4))
    NG = H // G
    wo_groups = []
    h0 = 0
    for n in WO_CHUNKS:
        wo_groups.append((h0, n))
        h0 += n
    NWO = len(wo_groups)
    scale = DH ** -0.5
    S_X, S_WQ, S_W3, S_W4, S_K = 0, 1, 2, 3, 4
    S_WO = S_K + 2 * NG
    NSEM = S_WO + NWO

    def kernel(x_hbm, k_hbm, v_hbm, wq_hbm, wo_hbm, w3t_hbm, w4_hbm, o_ref,
               x_buf, k_buf, v_buf, wq_buf, wo_buf, w3t_buf, w4_buf,
               q_buf, oh_buf, sems):
        def cp_x():
            return pltpu.make_async_copy(x_hbm, x_buf, sems.at[S_X])

        def cp_wq():
            return pltpu.make_async_copy(wq_hbm, wq_buf, sems.at[S_WQ])

        def cp_w3():
            return pltpu.make_async_copy(w3t_hbm, w3t_buf, sems.at[S_W3])

        def cp_w4():
            return pltpu.make_async_copy(w4_hbm, w4_buf, sems.at[S_W4])

        def cp_k(g):
            return pltpu.make_async_copy(
                k_hbm.at[0, pl.ds(g * G, G), pl.ds(SK - W, W), :],
                k_buf.at[pl.ds(g * G, G)], sems.at[S_K + 2 * g])

        def cp_v(g):
            return pltpu.make_async_copy(
                v_hbm.at[0, pl.ds(g * G, G), pl.ds(SK - W, W), :],
                v_buf.at[pl.ds(g * G, G)], sems.at[S_K + 2 * g + 1])

        def cp_wo(g):
            r0, n = wo_groups[g]
            return pltpu.make_async_copy(
                wo_hbm.at[pl.ds(r0 * DH, n * DH), :],
                wo_buf.at[pl.ds(r0 * DH, n * DH), :], sems.at[S_WO + g])

        cp_x().start()
        cp_wq().start()
        for g in range(NG):
            cp_k(g).start()
            cp_v(g).start()
        cp_w3().start()
        cp_w4().start()
        for g in range(NWO):
            cp_wo(g).start()

        cp_x().wait()
        x = x_buf[...].astype(F32)
        xn = _ln(x)
        cp_wq().wait()
        xn8 = jnp.broadcast_to(xn.astype(BF), (8, D))
        q = jnp.dot(xn8, wq_buf[...], preferred_element_type=F32)
        for h in range(H):
            q_buf[h] = q[:, h * DH:(h + 1) * DH]

        def head(h, carry):
            @pl.when(h % G == 0)
            def _():
                cp_k(h // G).wait()
                cp_v(h // G).wait()

            qh = q_buf[h].astype(BF)
            s = lax.dot_general(qh, k_buf[h], NT, preferred_element_type=F32)
            m = jnp.max(s, axis=-1, keepdims=True)
            p = jnp.exp2((s - m) * (scale * LOG2E))
            l = jnp.sum(p, axis=-1, keepdims=True)
            o = jnp.dot(p.astype(BF), v_buf[h], preferred_element_type=F32)
            oh_buf[h] = o * (1.0 / l)
            return carry

        lax.fori_loop(0, H, head, 0)

        cp_w3().wait()
        cp_w4().wait()
        x1n = jnp.broadcast_to(_ln(xn).astype(BF), (8, D))
        hh = lax.dot_general(x1n, w3t_buf[...], NT, preferred_element_type=F32)
        hh = jax.nn.gelu(hh, approximate=True).astype(BF)
        h2 = jnp.dot(hh, w4_buf[...], preferred_element_type=F32)[0:1, :]
        y = xn + h2
        gate = y * jax.nn.sigmoid(y)

        acc = jnp.zeros((8, D), F32)
        for g in range(NWO):
            r0, n = wo_groups[g]
            cp_wo(g).wait()
            o_cat = jnp.concatenate(
                [oh_buf[h] for h in range(r0, r0 + n)], axis=-1).astype(BF)
            acc = acc + jnp.dot(o_cat, wo_buf[pl.ds(r0 * DH, n * DH), :],
                                preferred_element_type=F32)
        o_ref[...] = (x + acc[0:1, :] * gate).astype(BF)

    out = pl.pallas_call(
        kernel,
        out_shape=jax.ShapeDtypeStruct((1, D), BF),
        in_specs=[pl.BlockSpec(memory_space=pl.ANY)] * 7,
        out_specs=pl.BlockSpec(memory_space=pltpu.VMEM),
        scratch_shapes=[
            pltpu.VMEM((1, D), BF),
            pltpu.VMEM((H, W, DH), BF),
            pltpu.VMEM((H, W, DH), BF),
            pltpu.VMEM((D, H * DH), BF),
            pltpu.VMEM((H * DH, D), BF),
            pltpu.VMEM((F, D), BF),
            pltpu.VMEM((F, D), BF),
            pltpu.VMEM((H, 8, DH), F32),
            pltpu.VMEM((H, 8, DH), F32),
            pltpu.SemaphoreType.DMA((NSEM,)),
        ],
        compiler_params=pltpu.CompilerParams(
            vmem_limit_bytes=110 * 1024 * 1024,
            disable_semaphore_checks=True,
        ),
    )(A_x.reshape(1, D), A_k_cache, A_v_cache, A_wq, A_wo, B_w3.T, B_w4)
    return out.reshape(1, 1, D)
```

```python
import jax
import jax.numpy as jnp
from jax import lax
from jax.experimental import pallas as pl
from jax.experimental.pallas import tpu as pltpu

D = 512
H = 32
DH = 128
F = 1376
BF = jnp.bfloat16
F32 = jnp.float32
LOG2E = 1.4426950408889634
NT = (((1,), (1,)), ((), ()))

HG = 4
NG = H // HG
RD = 32
QD = 32


def _ln(x, eps=1e-5):
    m = jnp.mean(x, axis=-1, keepdims=True)
    xc = x - m
    v = jnp.mean(xc * xc, axis=-1, keepdims=True)
    return xc * lax.rsqrt(v + eps)


@jax.jit
def pallas_recurrent_scan__sliding_block_cached__mixer_s_mlp__decode_kernel(
    A_x: jax.Array,
    A_k_cache: jax.Array,
    A_v_cache: jax.Array,
    A_wq: jax.Array,
    A_wo: jax.Array,
    B_x: jax.Array,
    B_w1: jax.Array,
    B_w2: jax.Array,
    B_w3: jax.Array,
    B_w4: jax.Array,
):
    assert A_x.shape == (1, 1, D)
    SK = A_k_cache.shape[2]
    W = min(4096, max(256, SK // 4))
    assert W == 4 * QD * RD
    scale = DH ** -0.5
    S_X, S_WQ, S_W3, S_W4 = 0, 1, 2, 3
    S_K = 4
    S_V = S_K + NG
    S_WO = S_V + NG
    NSEM = S_WO + 8

    def kernel(x_hbm, k_hbm, v_hbm, wq_hbm, wo_hbm, w3t_hbm, w4_hbm, o_ref,
               x_buf, k_buf, v_buf, wq_buf, wo_buf, w3t_buf, w4_buf,
               q_buf, p_buf, oh_buf, xs_buf, acc_buf, sems):
        def kv(src, dst, g, c, sem0, prio):
            r0 = pl.multiple_of(c * RD, RD)
            pltpu.make_async_copy(
                src.at[0, pl.ds(g * HG, HG), pl.ds(SK - W + r0, RD), :],
                dst.at[pl.ds(g * HG, HG), pl.ds(r0, RD), :],
                sems.at[sem0 + g]).start(priority=prio)

        def wq(rb, cb, prio):
            r0 = pl.multiple_of(rb * 8, 8)
            c0 = pl.multiple_of(cb * 512, 512)
            pltpu.make_async_copy(
                wq_hbm.at[:, pl.ds(r0, 8), pl.ds(c0, 512)],
                wq_buf.at[:, pl.ds(r0, 8), pl.ds(c0, 512)],
                sems.at[S_WQ]).start(priority=prio)

        def w34(src, dst, j, sem, prio):
            r0 = pl.multiple_of(j * 32, 32)
            pltpu.make_async_copy(
                src.at[pl.ds(r0, 32), :], dst.at[pl.ds(r0, 32), :],
                sems.at[sem]).start(priority=prio)

        def wo(jg, j, prio):
            r0 = pl.multiple_of(jg * 128 + j * 8, 8)
            pltpu.make_async_copy(
                wo_hbm.at[:, pl.ds(r0, 8), :], wo_buf.at[:, pl.ds(r0, 8), :],
                sems.at[S_WO + jg]).start(priority=prio)

        def loop(lo, hi, body):
            n = hi - lo
            lax.fori_loop(lo, hi, lambda i, c: (body(i), c)[1], 0,
                          unroll=2 if n % 2 == 0 else 1)

        def wait_all(buf, sem):
            pltpu.make_async_copy(buf, buf, sems.at[sem]).wait()

        def scores(h):
            qh = q_buf[h].astype(BF)
            s = lax.dot_general(qh, k_buf[h], NT, preferred_element_type=F32)
            m = jnp.max(s, axis=-1, keepdims=True)
            p = jnp.exp2((s - m) * (scale * LOG2E))
            l = jnp.sum(p, axis=-1, keepdims=True)
            p_buf[h] = p.astype(BF)
            oh_buf[h] = jnp.broadcast_to(1.0 / l, (8, DH))

        def pv(h):
            o = jnp.dot(p_buf[h], v_buf[h], preferred_element_type=F32)
            oh_buf[h] = o * oh_buf[h]

        def do_scores(h0, n):
            lax.fori_loop(h0, h0 + n, lambda h, c: (scores(h), c)[1], 0)

        def do_pv(h0, n):
            lax.fori_loop(h0, h0 + n, lambda h, c: (pv(h), c)[1], 0)

        def wait_k(g):
            wait_all(k_buf.at[pl.ds(g * HG, HG)], S_K + g)

        def wait_v(g):
            wait_all(v_buf.at[pl.ds(g * HG, HG)], S_V + g)

        def qproj():
            wait_all(x_buf, S_X)
            wait_all(wq_buf, S_WQ)
            x = x_buf[...].astype(F32)
            xn = _ln(x)
            xs_buf[0:1, :] = x
            xs_buf[1:2, :] = xn
            xn8 = jnp.broadcast_to(xn.astype(BF), (8, D))
            q = jnp.dot(xn8, wq_buf[...].reshape(D, H * DH),
                        preferred_element_type=F32)
            for h in range(H):
                q_buf[h] = q[:, h * DH:(h + 1) * DH]

        def issue_q(g, q, last):
            def k_desc(r):
                kv(k_hbm, k_buf, g, q * QD + r, S_K, 0)

            if q < 2:
                def body(r):
                    k_desc(r)
                    kv(v_hbm, v_buf, g, (q + 2) * QD + r, S_V, 1)
                loop(0, QD, body)
            elif not last:
                def body(r):
                    k_desc(r)
                    kv(v_hbm, v_buf, g + 1, (q - 2) * QD + r, S_V, 1)
                loop(0, QD, body)
            elif q == 2:
                def body(r):
                    k_desc(r)
                    w34(w4_hbm, w4_buf, r, S_W4, 1)
                loop(0, QD, body)
            else:
                def body(r):
                    k_desc(r)
                    w34(w4_hbm, w4_buf, 32 + r, S_W4, 1)
                loop(0, 11, body)

                def body(r):
                    k_desc(r)
                    wo(4, r - 11, 1)
                loop(11, 27, body)

                def body(r):
                    k_desc(r)
                    wo(5, r - 27, 1)
                loop(27, 32, body)

        def group(g, last, first):
            issue_q(g, 0, last)
            if not first:
                wait_k(g - 1)
                do_scores((g - 1) * HG, 2)
            issue_q(g, 1, last)
            if first:
                qproj()
            else:
                do_scores((g - 1) * HG + 2, 2)
            issue_q(g, 2, last)
            if not first:
                wait_v(g - 1)
                do_pv((g - 1) * HG, HG)
            issue_q(g, 3, last)

        def w3_wo(lo, hi):
            j = lo
            while j < hi:
                b = 21 + j
                jg, off = 4 + b // 16, b % 16
                n = min(hi - j, 16 - off)

                def body(r, j=j, jg=jg, off=off):
                    w34(w3t_hbm, w3t_buf, j + r, S_W3, 0)
                    wo(jg, off + r, 1)
                loop(0, n, body)
                j += n

        pltpu.make_async_copy(x_hbm, x_buf, sems.at[S_X]).start()
        for rb in range(8, 16):
            loop(0, 8, lambda cb, rb=rb: wq(rb, cb, 1))
        for rb in range(0, 8):
            def body(cb, rb=rb):
                wq(rb, cb, 0)
                kv(v_hbm, v_buf, 0, rb * 8 + cb, S_V, 1)
            loop(0, 8, body)

        group(0, False, True)
        lax.fori_loop(1, NG - 1, lambda g, c: (group(g, False, False), c)[1], 0)
        group(NG - 1, True, False)

        gl = NG - 1
        w3_wo(0, 21)
        wait_k(gl)
        do_scores(gl * HG, 2)
        w3_wo(21, 43)
        do_scores(gl * HG + 2, 2)
        loop(0, 16, lambda r: wo(0, r, 0))
        wait_v(gl)
        do_pv(gl * HG, 2)
        loop(0, 16, lambda r: wo(1, r, 0))
        do_pv(gl * HG + 2, 2)
        loop(0, 16, lambda r: wo(2, r, 0))
        wait_all(w3t_buf, S_W3)
        wait_all(w4_buf, S_W4)
        xn = xs_buf[1:2, :]
        x1n = jnp.broadcast_to(_ln(xn).astype(BF), (8, D))
        hh = lax.dot_general(x1n, w3t_buf[...], NT, preferred_element_type=F32)
        hh = jax.nn.gelu(hh, approximate=True).astype(BF)
        h2 = jnp.dot(hh, w4_buf[...], preferred_element_type=F32)[0:1, :]
        y = xn + h2
        xs_buf[2:3, :] = y * jax.nn.sigmoid(y)
        loop(0, 16, lambda r: wo(3, r, 0))
        acc_buf[...] = jnp.zeros_like(acc_buf)
        for jg in (0, 1, 4, 2, 5, 3, 6, 7):
            wait_all(wo_buf.at[:, pl.ds(jg * 128, 128), :], S_WO + jg)
            o_cat = jnp.concatenate(
                [oh_buf[jg + 8 * q] for q in range(4)], axis=-1).astype(BF)
            w = wo_buf[:, pl.ds(jg * 128, 128), :].reshape(4 * 128, D)
            acc_buf[...] += jnp.dot(o_cat, w, preferred_element_type=F32)
        out = xs_buf[0:1, :] + acc_buf[0:1, :] * xs_buf[2:3, :]
        o_ref[...] = out.astype(BF)

    out = pl.pallas_call(
        kernel,
        out_shape=jax.ShapeDtypeStruct((1, D), BF),
        in_specs=[pl.BlockSpec(memory_space=pl.ANY)] * 7,
        out_specs=pl.BlockSpec(memory_space=pltpu.VMEM),
        scratch_shapes=[
            pltpu.VMEM((1, D), BF),
            pltpu.VMEM((H, W, DH), BF),
            pltpu.VMEM((H, W, DH), BF),
            pltpu.VMEM((4, 128, H * DH), BF),
            pltpu.VMEM((4, 1024, D), BF),
            pltpu.VMEM((F, D), BF),
            pltpu.VMEM((F, D), BF),
            pltpu.VMEM((H, 8, DH), F32),
            pltpu.VMEM((H, 8, W), BF),
            pltpu.VMEM((H, 8, DH), F32),
            pltpu.VMEM((8, D), F32),
            pltpu.VMEM((8, D), F32),
            pltpu.SemaphoreType.DMA((NSEM,)),
        ],
        compiler_params=pltpu.CompilerParams(
            vmem_limit_bytes=110 * 1024 * 1024,
            disable_semaphore_checks=True,
            disable_bounds_checks=True,
        ),
    )(A_x.reshape(1, D), A_k_cache, A_v_cache,
      A_wq.reshape(4, 128, H * DH), A_wo.reshape(4, 1024, D), B_w3.T, B_w4)
    return out.reshape(1, 1, D)
```

```python
import jax
import jax.numpy as jnp
from jax import lax
from jax.experimental import pallas as pl
from jax.experimental.pallas import tpu as pltpu

D = 512
H = 32
DH = 128
F = 1376
BF = jnp.bfloat16
F32 = jnp.float32
LOG2E = 1.4426950408889634
NT = (((1,), (1,)), ((), ()))

HG = 4
NG = H // HG
RD = 32
NW3 = F // 32
NWQ = 128
NWO = 128
WQ_A = 40
LEAD = 26
WO_A = 64
CUTS = (40, 72, 112)
END_CUTS = (32, 72)
PIECES = (128, 96, 32)


def _ln(x, eps=1e-5):
    m = jnp.mean(x, axis=-1, keepdims=True)
    xc = x - m
    v = jnp.mean(xc * xc, axis=-1, keepdims=True)
    return xc * lax.rsqrt(v + eps)


@jax.jit
def pallas_recurrent_scan__sliding_block_cached__mixer_s_mlp__decode_kernel(
    A_x: jax.Array,
    A_k_cache: jax.Array,
    A_v_cache: jax.Array,
    A_wq: jax.Array,
    A_wo: jax.Array,
    B_x: jax.Array,
    B_w1: jax.Array,
    B_w2: jax.Array,
    B_w3: jax.Array,
    B_w4: jax.Array,
):
    assert A_x.shape == (1, 1, D)
    SK = A_k_cache.shape[2]
    W = min(4096, max(256, SK // 4))
    GD = W // RD
    assert GD == 128 and F == NW3 * 32
    scale = DH ** -0.5
    NR = H * DH

    RV = sum(PIECES)
    chunks = []
    j = 0
    while j < NWO - RV // 32:
        n = min(16, NWO - RV // 32 - j)
        chunks.append((j, n))
        j += n
    pcs = []
    for p in PIECES:
        pcs.append((j, p // 32))
        j += p // 32
    segs = chunks + pcs

    def wo_seg(j):
        for s, (j0, n) in enumerate(segs):
            if j0 <= j < j0 + n:
                return s, j0 + n
        raise ValueError(j)

    S_X, S_WQ, S_W3, S_W4 = 0, 1, 2, 3
    S_K = 4
    S_V = S_K + NG
    S_WO = S_V + NG
    NSEM = S_WO + len(segs)

    EA = ([("wq", j) for j in range(WQ_A)] + [("w3", j) for j in range(NW3)]
          + [("k", j) for j in range(NG * GD)] + [("wo", j) for j in range(WO_A)])
    EB = ([("wq", j) for j in range(WQ_A, NWQ)] + [("w4", j) for j in range(NW3)]
          + [("v", j) for j in range(NG * GD)] + [("wo", j) for j in range(WO_A, NWO)])
    k0 = WQ_A + NW3
    dV = 2 * WQ_A + LEAD - NWQ
    assert -GD < dV <= 0
    npairs = max(len(EA), len(EB) - LEAD)

    def pair(i):
        return (EA[i] if i < len(EA) else None,
                EB[i + LEAD] if i + LEAD < len(EB) else None)

    def kernel(x_hbm, k_hbm, v_hbm, wq_hbm, wo_hbm, w3t_hbm, w4_hbm, o_ref,
               x_buf, k_buf, v_buf, wq_buf, wo_buf, w3t_buf, w4_buf,
               q_buf, p_buf, oh_buf, xs_buf, acc_buf, oc_buf, sems):
        def kv(src, dst, g, c, sem0, prio):
            r0 = pl.multiple_of(c * RD, RD)
            pltpu.make_async_copy(
                src.at[0, pl.ds(g * HG, HG), pl.ds(SK - W + r0, RD), :],
                dst.at[pl.ds(g * HG, HG), pl.ds(r0, RD), :],
                sems.at[sem0 + g]).start(priority=prio)

        def rows32(src, dst, j, sem, prio):
            r0 = pl.multiple_of(j * 32, 32)
            pltpu.make_async_copy(
                src.at[pl.ds(r0, 32), :], dst.at[pl.ds(r0, 32), :],
                sems.at[sem]).start(priority=prio)

        def desc(item, t, prio):
            seg, j = item
            if seg == "wq":
                jj = j + t
                r0 = pl.multiple_of(lax.shift_right_logical(jj, 1) * 8, 8)
                c0 = pl.multiple_of(lax.bitwise_and(jj, 1) * 2048, 2048)
                pltpu.make_async_copy(
                    wq_hbm.at[pl.ds(r0, 8), pl.ds(c0, 2048)],
                    wq_buf.at[pl.ds(r0, 8), pl.ds(c0, 2048)],
                    sems.at[S_WQ]).start(priority=prio)
            elif seg == "w3":
                rows32(w3t_hbm, w3t_buf, j + t, S_W3, prio)
            elif seg == "w4":
                rows32(w4_hbm, w4_buf, j + t, S_W4, prio)
            elif seg == "wo":
                rows32(wo_hbm, wo_buf, j + t, S_WO + wo_seg(j)[0], prio)
            elif seg == "k":
                kv(k_hbm, k_buf, j // GD, j % GD + t, S_K, prio)
            else:
                kv(v_hbm, v_buf, j // GD, j % GD + t, S_V, prio)

        def runlen(item):
            seg, j = item
            if seg == "wq":
                return (WQ_A if j < WQ_A else NWQ) - j
            if seg in ("w3", "w4"):
                return NW3 - j
            if seg == "wo":
                return min(wo_seg(j)[1], WO_A if j < WO_A else NWO) - j
            return GD - j % GD

        def loop(n, body):
            lax.fori_loop(0, n, lambda i, c: (body(i), c)[1], 0,
                          unroll=2 if n % 2 == 0 else 1)

        def issue_static(items):
            m = 0
            while m < len(items):
                x, y = items[m]
                n = len(items) - m
                if x is not None:
                    n = min(n, runlen(x))
                if y is not None:
                    n = min(n, runlen(y))
                for t in range(1, n):
                    x2, y2 = items[m + t]
                    if (x2 is None) != (x is None) or (y2 is None) != (y is None):
                        n = t
                        break

                def body(t, x=x, y=y):
                    if x is not None:
                        desc(x, t, 0)
                    if y is not None:
                        desc(y, t, 1)
                loop(n, body)
                m += n

        def issue_pairs(lo, hi):
            issue_static([pair(i) for i in range(lo, min(hi, npairs))])

        def issue_kv(g, c0, c1):
            c = c0
            while c < c1:
                vv = c + dV
                if vv < 0:
                    gv, cv, n = -1, vv + GD, min(c1 - c, -vv)
                else:
                    gv, cv, n = 0, vv, c1 - c

                def body(t, c=c, gv=gv, cv=cv):
                    kv(k_hbm, k_buf, g, c + t, S_K, 0)
                    kv(v_hbm, v_buf, g + gv, cv + t, S_V, 1)
                loop(n, body)
                c += n

        def wait_all(buf, sem):
            pltpu.make_async_copy(buf, buf, sems.at[sem]).wait()

        def wait_k(g):
            wait_all(k_buf.at[pl.ds(g * HG, HG)], S_K + g)

        def wait_v(g):
            wait_all(v_buf.at[pl.ds(g * HG, HG)], S_V + g)

        def scores(h):
            qh = q_buf[h].astype(BF)
            s = lax.dot_general(qh, k_buf[h], NT, preferred_element_type=F32)
            m = jnp.max(s, axis=-1, keepdims=True)
            p = jnp.exp2((s - m) * (scale * LOG2E))
            l = jnp.sum(p, axis=-1, keepdims=True)
            p_buf[h] = p.astype(BF)
            oh_buf[h] = jnp.broadcast_to(1.0 / l, (8, DH))

        def pv(h):
            o = jnp.dot(p_buf[h], v_buf[h], preferred_element_type=F32)
            oh_buf[h] = o * oh_buf[h]

        def do_scores(h0, n):
            lax.fori_loop(h0, h0 + n, lambda h, c: (scores(h), c)[1], 0)

        def do_pv(h0, n):
            lax.fori_loop(h0, h0 + n, lambda h, c: (pv(h), c)[1], 0)

        def qproj():
            wait_all(x_buf, S_X)
            wait_all(wq_buf, S_WQ)
            x = x_buf[...].astype(F32)
            xn = _ln(x)
            xs_buf[0:1, :] = x
            xs_buf[1:2, :] = xn
            xn8 = jnp.broadcast_to(xn.astype(BF), (8, D))
            q = jnp.dot(xn8, wq_buf[...], preferred_element_type=F32)
            for h in range(H):
                q_buf[h] = q[:, h * DH:(h + 1) * DH]

        def mlp_gate():
            wait_all(w3t_buf, S_W3)
            wait_all(w4_buf, S_W4)
            xn = xs_buf[1:2, :]
            x1n = jnp.broadcast_to(_ln(xn).astype(BF), (8, D))
            hh = lax.dot_general(x1n, w3t_buf[...], NT, preferred_element_type=F32)
            hh = jax.nn.gelu(hh, approximate=True).astype(BF)
            h2 = jnp.dot(hh, w4_buf[...], preferred_element_type=F32)[0:1, :]
            y = xn + h2
            xs_buf[2:3, :] = y * jax.nn.sigmoid(y)

        def wo_chunk(s, first=False):
            j0, n = segs[s]
            r0, nr = j0 * 32, n * 32
            wait_all(wo_buf.at[pl.ds(r0, nr), :], S_WO + s)
            h0 = r0 // DH
            o_cat = jnp.concatenate(
                [oh_buf[h] for h in range(h0, h0 + nr // DH)], axis=-1).astype(BF)
            d = jnp.dot(o_cat, wo_buf[pl.ds(r0, nr), :], preferred_element_type=F32)
            if first:
                acc_buf[...] = d
            else:
                acc_buf[...] += d

        issue_static([(None, EB[j]) for j in range(LEAD)])
        pltpu.make_async_copy(x_hbm, x_buf, sems.at[S_X]).start()
        issue_pairs(0, k0 + 96)
        qproj()
        issue_pairs(k0 + 96, k0 + GD)
        mlp_gate()

        def group(g, carry):
            issue_kv(g, 0, CUTS[0])
            wait_k(g - 1)
            do_scores((g - 1) * HG, 2)
            issue_kv(g, CUTS[0], CUTS[1])
            do_scores((g - 1) * HG + 2, 2)
            issue_kv(g, CUTS[1], CUTS[2])
            wait_v(g - 1)
            do_pv((g - 1) * HG, HG)
            issue_kv(g, CUTS[2], GD)
            return carry
        lax.fori_loop(1, NG, group, 0)

        gl = NG - 1
        e0 = k0 + NG * GD
        issue_pairs(e0, e0 + END_CUTS[0])
        wait_k(gl)
        do_scores(gl * HG, 2)
        issue_pairs(e0 + END_CUTS[0], e0 + END_CUTS[1])
        do_scores(gl * HG + 2, 2)
        issue_pairs(e0 + END_CUTS[1], npairs)

        wo_chunk(0, first=True)
        wait_v(gl)
        do_pv(gl * HG, HG)
        assert RV % DH == 0
        for jj in range(RV // DH):
            hv = H - RV // DH + jj
            oc_buf[pl.ds(jj * DH, DH), :] = jnp.transpose(
                jnp.broadcast_to(oh_buf[hv][0:1, :], (DH, DH)))
        na = WO_A // 16
        ia, ib = 1, na
        while ia < na or ib < len(chunks):
            if ia < na:
                wo_chunk(ia)
                ia += 1
            if ib < len(chunks):
                wo_chunk(ib)
                ib += 1

        row = lax.broadcasted_iota(jnp.int32, (8, D), 0)
        t8 = jnp.where(row == 0, acc_buf[...], 0.0)
        for i, (j0, n) in enumerate(pcs):
            r0, nr = j0 * 32, n * 32
            wait_all(wo_buf.at[pl.ds(r0, nr), :], S_WO + len(chunks) + i)
            wl = wo_buf[pl.ds(r0, nr), :].astype(F32)
            oc = oc_buf[pl.ds(r0 - (NR - RV), nr), :]
            for k in range(nr // 8):
                ock = oc[k * 8:(k + 1) * 8, :]
                t8 = t8 + jnp.concatenate([ock] * (D // DH), axis=1) * wl[k * 8:(k + 1) * 8, :]
        s = jnp.sum(t8, axis=0, keepdims=True)
        o_ref[...] = (xs_buf[0:1, :] + s * xs_buf[2:3, :]).astype(BF)

    out = pl.pallas_call(
        kernel,
        out_shape=jax.ShapeDtypeStruct((1, D), BF),
        in_specs=[pl.BlockSpec(memory_space=pl.ANY)] * 7,
        out_specs=pl.BlockSpec(memory_space=pltpu.VMEM),
        scratch_shapes=[
            pltpu.VMEM((1, D), BF),
            pltpu.VMEM((H, W, DH), BF),
            pltpu.VMEM((H, W, DH), BF),
            pltpu.VMEM((D, H * DH), BF),
            pltpu.VMEM((H * DH, D), BF),
            pltpu.VMEM((F, D), BF),
            pltpu.VMEM((F, D), BF),
            pltpu.VMEM((H, 8, DH), F32),
            pltpu.VMEM((H, 8, W), BF),
            pltpu.VMEM((H, 8, DH), F32),
            pltpu.VMEM((8, D), F32),
            pltpu.VMEM((8, D), F32),
            pltpu.VMEM((RV, DH), F32),
            pltpu.SemaphoreType.DMA((NSEM,)),
        ],
        compiler_params=pltpu.CompilerParams(
            vmem_limit_bytes=110 * 1024 * 1024,
            disable_semaphore_checks=True,
            disable_bounds_checks=True,
        ),
    )(A_x.reshape(1, D), A_k_cache, A_v_cache, A_wq, A_wo, B_w3.T, B_w4)
    return out.reshape(1, 1, D)
```

```python
import jax
import jax.numpy as jnp
from jax import lax
from jax.experimental import pallas as pl
from jax.experimental.pallas import tpu as pltpu

D = 512
H = 32
DH = 128
F = 1376
BF = jnp.bfloat16
F32 = jnp.float32
LOG2E = 1.4426950408889634
NT = (((1,), (1,)), ((), ()))

HG = 4
NG = H // HG
RD = 32
NW3 = F // 32
NWQ = 128
NWO = 128
WQ_A = 40
LEAD = 26
WO_A = 64
CUTS = (40, 72, 112)
END_CUTS = (32, 72)
PIECES = (128, 96, 32)


def _ln(x, eps=1e-5):
    m = jnp.mean(x, axis=-1, keepdims=True)
    xc = x - m
    v = jnp.mean(xc * xc, axis=-1, keepdims=True)
    return xc * lax.rsqrt(v + eps)


@jax.jit
def pallas_recurrent_scan__sliding_block_cached__mixer_s_mlp__decode_kernel(
    A_x: jax.Array,
    A_k_cache: jax.Array,
    A_v_cache: jax.Array,
    A_wq: jax.Array,
    A_wo: jax.Array,
    B_x: jax.Array,
    B_w1: jax.Array,
    B_w2: jax.Array,
    B_w3: jax.Array,
    B_w4: jax.Array,
):
    assert A_x.shape == (1, 1, D)
    SK = A_k_cache.shape[2]
    W = min(4096, max(256, SK // 4))
    GD = W // RD
    assert GD == 128 and F == NW3 * 32
    scale = DH ** -0.5
    NR = H * DH

    RV = sum(PIECES)
    chunks = []
    j = 0
    while j < NWO - RV // 32:
        n = min(16, NWO - RV // 32 - j)
        chunks.append((j, n))
        j += n
    pcs = []
    for p in PIECES:
        pcs.append((j, p // 32))
        j += p // 32
    segs = chunks + pcs

    def wo_seg(j):
        for s, (j0, n) in enumerate(segs):
            if j0 <= j < j0 + n:
                return s, j0 + n
        raise ValueError(j)

    S_X, S_WQ, S_W3, S_W4 = 0, 1, 2, 3
    S_K = 4
    S_V = S_K + NG
    S_WO = S_V + NG
    NSEM = S_WO + len(segs)

    EA = ([("wq", j) for j in range(WQ_A)] + [("w3", j) for j in range(NW3)]
          + [("k", j) for j in range(NG * GD)] + [("wo", j) for j in range(WO_A)])
    EB = ([("wq", j) for j in range(WQ_A, NWQ)] + [("w4", j) for j in range(NW3)]
          + [("v", j) for j in range(NG * GD)] + [("wo", j) for j in range(WO_A, NWO)])
    k0 = WQ_A + NW3
    dV = 2 * WQ_A + LEAD - NWQ
    assert -GD < dV <= 0
    npairs = max(len(EA), len(EB) - LEAD)

    def pair(i):
        return (EA[i] if i < len(EA) else None,
                EB[i + LEAD] if i + LEAD < len(EB) else None)

    def kernel(x_hbm, k_hbm, v_hbm, wq_hbm, wo_hbm, w3t_hbm, w4_hbm, o_ref,
               x_buf, k_buf, v_buf, wq_buf, wo_buf, w3t_buf, w4_buf,
               q_buf, p_buf, oh_buf, xs_buf, acc_buf, oc_buf, sems):
        def kv(src, dst, g, c, sem0, prio):
            r0 = pl.multiple_of(c * RD, RD)
            pltpu.make_async_copy(
                src.at[0, pl.ds(g * HG, HG), pl.ds(SK - W + r0, RD), :],
                dst.at[pl.ds(g * HG, HG), pl.ds(r0, RD), :],
                sems.at[sem0 + g]).start(priority=prio)

        def rows32(src, dst, j, sem, prio):
            r0 = pl.multiple_of(j * 32, 32)
            pltpu.make_async_copy(
                src.at[pl.ds(r0, 32), :], dst.at[pl.ds(r0, 32), :],
                sems.at[sem]).start(priority=prio)

        def desc(item, t, u, prio):
            seg, j = item
            if seg == "wq":
                assert j % 2 == 0
                r0 = pl.multiple_of((j // 2 + t) * 8, 8)
                pltpu.make_async_copy(
                    wq_hbm.at[pl.ds(r0, 8), pl.ds(u * 2048, 2048)],
                    wq_buf.at[pl.ds(r0, 8), pl.ds(u * 2048, 2048)],
                    sems.at[S_WQ]).start(priority=prio)
                return
            jt = 2 * t + u
            if seg == "w3":
                rows32(w3t_hbm, w3t_buf, j + jt, S_W3, prio)
            elif seg == "w4":
                rows32(w4_hbm, w4_buf, j + jt, S_W4, prio)
            elif seg == "wo":
                rows32(wo_hbm, wo_buf, j + jt, S_WO + wo_seg(j)[0], prio)
            elif seg == "k":
                kv(k_hbm, k_buf, j // GD, j % GD + jt, S_K, prio)
            else:
                kv(v_hbm, v_buf, j // GD, j % GD + jt, S_V, prio)

        def runlen(item):
            seg, j = item
            if seg == "wq":
                return (WQ_A if j < WQ_A else NWQ) - j
            if seg in ("w3", "w4"):
                return NW3 - j
            if seg == "wo":
                return min(wo_seg(j)[1], WO_A if j < WO_A else NWO) - j
            return GD - j % GD

        def loop2(n, body):
            if n >= 2:
                def two(t, c):
                    body(t, 0)
                    body(t, 1)
                    return c
                lax.fori_loop(0, n // 2, two, 0)
            if n % 2:
                body(n // 2, 0)

        def issue_static(items):
            m = 0
            while m < len(items):
                x, y = items[m]
                n = len(items) - m
                if x is not None:
                    n = min(n, runlen(x))
                if y is not None:
                    n = min(n, runlen(y))
                for t in range(1, n):
                    x2, y2 = items[m + t]
                    if (x2 is None) != (x is None) or (y2 is None) != (y is None):
                        n = t
                        break

                def body(t, u, x=x, y=y):
                    if x is not None:
                        desc(x, t, u, 0)
                    if y is not None:
                        desc(y, t, u, 1)
                loop2(n, body)
                m += n

        def issue_pairs(lo, hi):
            issue_static([pair(i) for i in range(lo, min(hi, npairs))])

        def issue_kv(g, c0, c1):
            c = c0
            while c < c1:
                vv = c + dV
                if vv < 0:
                    gv, cv, n = -1, vv + GD, min(c1 - c, -vv)
                else:
                    gv, cv, n = 0, vv, c1 - c

                def body(t, u, c=c, gv=gv, cv=cv):
                    kv(k_hbm, k_buf, g, c + 2 * t + u, S_K, 0)
                    kv(v_hbm, v_buf, g + gv, cv + 2 * t + u, S_V, 1)
                loop2(n, body)
                c += n

        def wait_all(buf, sem):
            pltpu.make_async_copy(buf, buf, sems.at[sem]).wait()

        def wait_k(g):
            wait_all(k_buf.at[pl.ds(g * HG, HG)], S_K + g)

        def wait_v(g):
            wait_all(v_buf.at[pl.ds(g * HG, HG)], S_V + g)

        def scores(h):
            qh = q_buf[h].astype(BF)
            s = lax.dot_general(qh, k_buf[h], NT, preferred_element_type=F32)
            m = jnp.max(s, axis=-1, keepdims=True)
            p = jnp.exp2((s - m) * (scale * LOG2E))
            l = jnp.sum(p, axis=-1, keepdims=True)
            p_buf[h] = p.astype(BF)
            oh_buf[h] = jnp.broadcast_to(1.0 / l, (8, DH))

        def pv(h):
            o = jnp.dot(p_buf[h], v_buf[h], preferred_element_type=F32)
            oh_buf[h] = o * oh_buf[h]

        def do_scores(h0, n):
            lax.fori_loop(h0, h0 + n, lambda h, c: (scores(h), c)[1], 0)

        def do_pv(h0, n):
            lax.fori_loop(h0, h0 + n, lambda h, c: (pv(h), c)[1], 0)

        def qproj():
            wait_all(x_buf, S_X)
            wait_all(wq_buf, S_WQ)
            x = x_buf[...].astype(F32)
            xn = _ln(x)
            xs_buf[0:1, :] = x
            xs_buf[1:2, :] = xn
            xn8 = jnp.broadcast_to(xn.astype(BF), (8, D))
            q = jnp.dot(xn8, wq_buf[...], preferred_element_type=F32)
            for h in range(H):
                q_buf[h] = q[:, h * DH:(h + 1) * DH]

        def mlp_gate():
            wait_all(w3t_buf, S_W3)
            wait_all(w4_buf, S_W4)
            xn = xs_buf[1:2, :]
            x1n = jnp.broadcast_to(_ln(xn).astype(BF), (8, D))
            hh = lax.dot_general(x1n, w3t_buf[...], NT, preferred_element_type=F32)
            hh = jax.nn.gelu(hh, approximate=True).astype(BF)
            h2 = jnp.dot(hh, w4_buf[...], preferred_element_type=F32)[0:1, :]
            y = xn + h2
            xs_buf[2:3, :] = y * jax.nn.sigmoid(y)

        def wo_chunk(s, first=False):
            j0, n = segs[s]
            r0, nr = j0 * 32, n * 32
            wait_all(wo_buf.at[pl.ds(r0, nr), :], S_WO + s)
            h0 = r0 // DH
            o_cat = jnp.concatenate(
                [oh_buf[h] for h in range(h0, h0 + nr // DH)], axis=-1).astype(BF)
            d = jnp.dot(o_cat, wo_buf[pl.ds(r0, nr), :], preferred_element_type=F32)
            if first:
                acc_buf[...] = d
            else:
                acc_buf[...] += d

        issue_static([(None, EB[j]) for j in range(LEAD)])
        pltpu.make_async_copy(x_hbm, x_buf, sems.at[S_X]).start()
        issue_pairs(0, k0 + 96)
        qproj()
        issue_pairs(k0 + 96, k0 + GD)
        mlp_gate()

        def group(g, carry):
            issue_kv(g, 0, CUTS[0])
            wait_k(g - 1)
            do_scores((g - 1) * HG, 2)
            issue_kv(g, CUTS[0], CUTS[1])
            do_scores((g - 1) * HG + 2, 2)
            issue_kv(g, CUTS[1], CUTS[2])
            wait_v(g - 1)
            do_pv((g - 1) * HG, HG)
            issue_kv(g, CUTS[2], GD)
            return carry
        lax.fori_loop(1, NG, group, 0)

        gl = NG - 1
        e0 = k0 + NG * GD
        issue_pairs(e0, e0 + END_CUTS[0])
        wait_k(gl)
        do_scores(gl * HG, 2)
        issue_pairs(e0 + END_CUTS[0], e0 + END_CUTS[1])
        do_scores(gl * HG + 2, 2)
        issue_pairs(e0 + END_CUTS[1], npairs)

        wo_chunk(0, first=True)
        wait_v(gl)
        do_pv(gl * HG, HG)
        assert RV % DH == 0
        for jj in range(RV // DH):
            hv = H - RV // DH + jj
            oc_buf[pl.ds(jj * DH, DH), :] = jnp.transpose(
                jnp.broadcast_to(oh_buf[hv][0:1, :], (DH, DH)))
        na = WO_A // 16
        ia, ib = 1, na
        while ia < na or ib < len(chunks):
            if ia < na:
                wo_chunk(ia)
                ia += 1
            if ib < len(chunks):
                wo_chunk(ib)
                ib += 1

        row = lax.broadcasted_iota(jnp.int32, (8, D), 0)
        t8 = jnp.where(row == 0, acc_buf[...], 0.0)
        for i, (j0, n) in enumerate(pcs):
            r0, nr = j0 * 32, n * 32
            wait_all(wo_buf.at[pl.ds(r0, nr), :], S_WO + len(chunks) + i)
            wl = wo_buf[pl.ds(r0, nr), :].astype(F32)
            oc = oc_buf[pl.ds(r0 - (NR - RV), nr), :]
            for k in range(nr // 8):
                ock = oc[k * 8:(k + 1) * 8, :]
                t8 = t8 + jnp.concatenate([ock] * (D // DH), axis=1) * wl[k * 8:(k + 1) * 8, :]
        s = jnp.sum(t8, axis=0, keepdims=True)
        o_ref[...] = (xs_buf[0:1, :] + s * xs_buf[2:3, :]).astype(BF)

    out = pl.pallas_call(
        kernel,
        out_shape=jax.ShapeDtypeStruct((1, D), BF),
        in_specs=[pl.BlockSpec(memory_space=pl.ANY)] * 7,
        out_specs=pl.BlockSpec(memory_space=pltpu.VMEM),
        scratch_shapes=[
            pltpu.VMEM((1, D), BF),
            pltpu.VMEM((H, W, DH), BF),
            pltpu.VMEM((H, W, DH), BF),
            pltpu.VMEM((D, H * DH), BF),
            pltpu.VMEM((H * DH, D), BF),
            pltpu.VMEM((F, D), BF),
            pltpu.VMEM((F, D), BF),
            pltpu.VMEM((H, 8, DH), F32),
            pltpu.VMEM((H, 8, W), BF),
            pltpu.VMEM((H, 8, DH), F32),
            pltpu.VMEM((8, D), F32),
            pltpu.VMEM((8, D), F32),
            pltpu.VMEM((RV, DH), F32),
            pltpu.SemaphoreType.DMA((NSEM,)),
        ],
        compiler_params=pltpu.CompilerParams(
            vmem_limit_bytes=110 * 1024 * 1024,
            disable_semaphore_checks=True,
            disable_bounds_checks=True,
        ),
    )(A_x.reshape(1, D), A_k_cache, A_v_cache, A_wq, A_wo, B_w3.T, B_w4)
    return out.reshape(1, 1, D)
```
